```python
import os as _os
_os.environ.setdefault("JAX_PLATFORMS", "cpu")
import jax
import jax.numpy as jnp

def _softmax(x, axis=-1):
    return jax.nn.softmax(x, axis=axis)
def _gelu(x):
    return jax.nn.gelu(x, approximate=True)
def _silu(x):
    return jax.nn.silu(x)
def _sigmoid(x):
    return jax.nn.sigmoid(x)
def _layernorm(x, axis=-1, eps=1e-5):
    m = jnp.mean(x, axis=axis, keepdims=True)
    v = jnp.var(x, axis=axis, keepdims=True)
    return (x - m) / jnp.sqrt(v + eps)
def _scatter_add(tgt, idx, src, axis=0):
    return tgt.at[idx].add(src)
def _segment_sum(src, seg, n):
    return jax.ops.segment_sum(src, seg, n)
class _Rng:
    def __init__(self, key):
        self._k = key
    def _next(self):
        self._k, sub = jax.random.split(self._k)
        return sub
    def normal(self, shape):
        return jax.random.normal(self._next(), shape, dtype=jnp.bfloat16)
    def randint(self, lo, hi, shape):
        return jax.random.randint(self._next(), shape, lo, hi, dtype=jnp.int32)
    def uniform(self, shape, lo=0.0, hi=1.0):
        return jax.random.uniform(self._next(), shape, jnp.bfloat16, lo, hi)
    def permutation(self, n):
        return jax.random.permutation(self._next(), n)


kernel_name = 'interleave_layers__sliding_local_dilated__mixer_channel_mlp__prompt'

def setup_inputs():
    _rng = _Rng(jax.random.key(int.from_bytes(__import__("os").urandom(4), "little")))
    _w = (lambda a: (lambda t: t.astype(jnp.bfloat16) if jnp.issubdtype(t.dtype, jnp.floating) else t)(jnp.asarray(a)))
    def _A_setup():
        B, S, D = 1, 2048, 512
        return {
            "x": _w((lambda *s: _rng.normal(s) * 0.05)(B, S, D)),
            "wqkv": _w((lambda *s: _rng.normal(s) * 0.05)(D, 3 * D)),
            "wo": _w((lambda *s: _rng.normal(s) * 0.05)(D, D)),
        }
    _A_in = _A_setup()

    def _B_setup():
        B, S, D, F = 1, 2048, 512, 1376
        return {
            "x": _w((lambda *s: _rng.normal(s) * 0.05)(B, S, D)),
            "w1": _w((lambda *s: _rng.normal(s) * 0.4)(D, F) * (D ** -0.5)),
            "b1": _w((lambda *s: _rng.normal(s) * 0.4)(F)),
            "w2": _w((lambda *s: _rng.normal(s) * 0.4)(F, D) * (F ** -0.5)),
            "b2": _w((lambda *s: _rng.normal(s) * 0.4)(D)),
        }
    _B_in = _B_setup()

    return {
        "A_x": _A_in["x"],
        "A_wqkv": _A_in["wqkv"],
        "A_wo": _A_in["wo"],
        "B_x": _B_in["x"],
        "B_w1": _B_in["w1"],
        "B_b1": _B_in["b1"],
        "B_w2": _B_in["w2"],
        "B_b2": _B_in["b2"],
    }

def reference(A_x, A_wqkv, A_wo, B_x, B_w1, B_b1, B_w2, B_b2):
    def _A_ref(x, wqkv, wo):
        B, S, D = x.shape
        H = 32; Dh = D // H
        W, dil = 8, 2
        qkv = (lambda x, *d: x.transpose(*d))((x @ wqkv).reshape(B, S, 3, H, Dh), 2, 0, 3, 1, 4)
        q, k, v = qkv[0], qkv[1], qkv[2]
        scale = Dh ** -0.5
        pos = jnp.arange(S)
        off = jnp.arange(W) * dil
        idx = pos[:, None] - off[None, :]
        mask = idx >= 0
        idx_c = jnp.where(mask, idx, 0).reshape(-1)
        kg = k[:, :, idx_c, :].reshape(B, H, S, W, Dh)
        vg = v[:, :, idx_c, :].reshape(B, H, S, W, Dh)
        logits = jnp.einsum("bhsd,bhswd->bhsw", q, kg) * scale
        logits = jnp.where(mask[None, None, :, :], logits, -1e9)
        attn = _softmax(logits, axis=-1)
        o = jnp.einsum("bhsw,bhswd->bhsd", attn, vg)
        return (lambda x, *d: x.transpose(*d))(o, 0, 2, 1, 3).reshape(B, S, D) @ wo

    def _B_ref(x, w1, b1, w2, b2):
        y = _layernorm(x, axis=-1)
        h = _gelu(jnp.einsum("bsd,df->bsf", y, w1) + b1)
        return jnp.einsum("bsf,fd->bsd", h, w2) + b2

    x = A_x
    x = x + _A_ref(_layernorm(x, axis=-1), A_wqkv, A_wo)
    x = x + _B_ref(_layernorm(x, axis=-1), B_w1, B_b1, B_w2, B_b2)
    x = x + _A_ref(_layernorm(x, axis=-1), A_wqkv, A_wo)
    x = x + _B_ref(_layernorm(x, axis=-1), B_w1, B_b1, B_w2, B_b2)
    return x
```

```python
import os
import jax
import jax.numpy as jnp
import jax.experimental.pallas as pl
import jax.experimental.pallas.tpu as pltpu

S, D, F = 2048, 512, 1376
H, DH, W, DIL = 32, 16, 8, 2
HALO = 16
T = 256
HT = T // 2
NT = S // T
RC = 16
PITCH = 20
EPS = 1e-5
F32 = jnp.float32
BF16 = jnp.bfloat16
U32 = jnp.uint32
NT_DIMS = (((1,), (1,)), ((), ()))

QCUTS = (0, 64, 128, 256)
W1CUTS = [int(v) for v in os.environ.get("W1CUTS", "0,512,1376").split(",")]
STAGE_P = os.environ.get("STAGE_P", "0123")
STAGE_L = os.environ.get("STAGE_L", "23")
STAGE_E = os.environ.get("STAGE_E", "")
OPT = os.environ.get("OPT", "").split(",")
NITER = int(os.environ.get("NITER", NT - 2))


def _ln(x):
    m = jnp.mean(x, axis=-1, keepdims=True)
    xc = x - m
    v = jnp.mean(xc * xc, axis=-1, keepdims=True)
    return xc * jax.lax.rsqrt(v + EPS)


def _gelu(x):
    c = 0.7978845608028654
    return 0.5 * x * (1.0 + jnp.tanh(c * (x + 0.044715 * (x * x * x))))


def _pack(x):
    return pltpu.bitcast(x, U32)


def _unpack(x):
    return pltpu.bitcast(x, BF16)


def _dot(a, b):
    return jnp.dot(a, b, preferred_element_type=F32)


def _dot_nt(a, b):
    return jax.lax.dot_general(a, b, NT_DIMS, preferred_element_type=F32)


def _kernel(x_hbm, wqkv_hbm, wo_hbm, w1t_hbm, b1_hbm, w2_hbm, b2_hbm, out_hbm,
            xin, wraw, woraw, wt32, wqkv_t, wqkv_n, wo_p, w1_s, w2_s, w1_p, w2_p,
            b1_s, b2_s, b1f, b2f, k_s, v_s, q_s, l_s, a_s, xres, xn_s, o_s,
            sem_in, sem_out):
    def cp(src, dst, i):
        return pltpu.make_async_copy(src, dst, sem_in.at[i])

    c_wv = [cp(wqkv_hbm.at[pl.ds(c * 256, 256), pl.ds(2 * D, D)],
               wraw.at[2, pl.ds(c * 256, 256), :], c) for c in range(2)]
    c_x0 = cp(x_hbm.at[pl.ds(0, T), :], xin.at[pl.ds(0, T), :], 2)
    c_wk = cp(wqkv_hbm.at[:, pl.ds(D, D)], wraw.at[1], 3)
    c_x1 = cp(x_hbm.at[pl.ds(T, T), :], xin.at[pl.ds(T, T), :], 3)
    c_wq = cp(wqkv_hbm.at[:, pl.ds(0, D)], wraw.at[0], 4)
    c_wo = cp(wo_hbm, woraw, 4)
    c_b1 = cp(b1_hbm, b1_s, 4)
    c_b2 = cp(b2_hbm, b2_s, 4)
    c_w1 = cp(w1t_hbm, w1_s, 5)
    c_w2 = cp(w2_hbm, w2_s, 5)
    c_xr = cp(x_hbm.at[pl.ds(2 * T, S - 2 * T), :], xin.at[pl.ds(2 * T, S - 2 * T), :], 6)
    for c in c_wv + [c_x0, c_wk, c_x1, c_wq, c_wo, c_b1, c_b2, c_w1, c_w2, c_xr]:
        c.start()

    def rows(tile, n=T, off=0):
        r0 = tile * T
        if not isinstance(tile, int):
            r0 = pl.multiple_of(r0, T)
        return pl.ds(r0 + off, n)

    def out_copy(rr):
        return pltpu.make_async_copy(o_s.at[rr, :], out_hbm.at[rr, :], sem_out.at[0])

    def gather_heads(buf, c, d):
        return wt32[buf, c, pl.ds(d, H, stride=PITCH), :]

    def scatter_heads(buf, c, wt):
        for h in range(H):
            wt32[buf, c, h * PITCH:h * PITCH + DH, :] = wt[h * DH:(h + 1) * DH, :]

    def permute_qkv(p, buf, chunks=range(4)):
        for c in chunks:
            scatter_heads(buf, c, wraw[p, c * 128:(c + 1) * 128, :].astype(F32).T)
        for d in range(DH):
            for c in chunks:
                blk = gather_heads(buf, c, d)
                if p == 0:
                    blk = blk * (DH ** -0.5)
                wqkv_t[p, d * H // 2:(d + 1) * H // 2, c * 128:(c + 1) * 128] = _pack(blk.astype(BF16))

    def permute_wo(buf):
        for c in range(4):
            scatter_heads(buf, c, woraw[:, c * 128:(c + 1) * 128].astype(F32))
        for d in range(DH):
            for c in range(4):
                wo_p[d * H // 2:(d + 1) * H // 2, c * 128:(c + 1) * 128] = _pack(
                    gather_heads(buf, c, d).astype(BF16))

    def proj(xn, p, first):
        if first or p == 1:
            return _dot_nt(xn, _unpack(wqkv_t[p]))
        return _dot(xn, _unpack(wqkv_n[p // 2]))

    def proj_kv(xn, p, slot, r0=0, r1=T, first=False):
        dst = k_s if p == 1 else v_s
        y = proj(xn[r0:r1], p, first)
        for t in range(4):
            dst[slot, t, HALO + r0:HALO + r1, :] = y[:, 128 * t:128 * (t + 1)]

    def proj_q(xn, slot, r0, r1, first=False):
        q_s[slot, r0:r1, :] = proj(xn[r0:r1], 0, first)

    def attention(slot, tile, stage, r0=0, r1=T):
        def through(i, w, r, val):
            if str(i) not in stage:
                return val
            l_s[i, w, r:r + RC, :] = val
            return l_s[i, w, r:r + RC, :]

        for r in range(r0, r1, RC):
            q = [q_s[slot, r:r + RC, 128 * t:128 * (t + 1)] for t in range(4)]
            logits = []
            for w in range(W):
                st = HALO + r - DIL * w
                p = q[0] * k_s[slot, 0, st:st + RC, :]
                for t in range(1, 4):
                    p = p + q[t] * k_s[slot, t, st:st + RC, :]
                p = through(0, w, r, p)
                p = p + pltpu.roll(p, 64, 1)
                p = through(1, w, r, p)
                p = p + pltpu.roll(p, 32, 1)
                if tile is not None and r < HALO and w > 0:
                    row = tile * T + r + jax.lax.broadcasted_iota(jnp.int32, (RC, 128), 0)
                    p = jnp.where(row >= DIL * w, p, -1e9)
                logits.append(through(2, w, r, p))
            m = logits[0]
            for w in range(1, W):
                m = jnp.maximum(m, logits[w])
            e = [through(3, w, r, jnp.exp(logits[w] - m)) for w in range(W)]
            den = e[0]
            for w in range(1, W):
                den = den + e[w]
            inv = 1.0 / den
            for t in range(4):
                acc = None
                for w in range(W):
                    st = HALO + r - DIL * w
                    term = e[w] * v_s[slot, t, st:st + RC, :]
                    acc = term if acc is None else acc + term
                a_s[slot, r // 2:(r + RC) // 2, 128 * t:128 * (t + 1)] = _pack((acc * inv).astype(BF16))

    def attn_out(x, slot, r0=0, r1=T):
        return x + _dot(_unpack(a_s[slot, r0 // 2:r1 // 2, :]), _unpack(wo_p[...]))

    def ln2(x):
        return _ln(_ln(x)).astype(BF16)

    def mlp1(y, a=0, b=F, first=False):
        w = w1_s[a:b, :] if first else _unpack(w1_p[a // 2:b // 2, :])
        return _gelu(_dot_nt(y, w) + b1f[:, a:b]).astype(BF16)

    def mlp2(x, h, a=0, b=D, first=False):
        w = w2_s[:, a:b] if first else _unpack(w2_p[:, a:b])
        return x[:, a:b] + _dot(h, w) + b2f[:, a:b]

    def load_x(rr):
        return xin[rr, :].astype(F32)

    def set_halo(slot, src_slot):
        k_s[slot, :, 0:HALO, :] = k_s[src_slot, :, T:T + HALO, :]
        v_s[slot, :, 0:HALO, :] = v_s[src_slot, :, T:T + HALO, :]

    zeros = jnp.zeros((4, HALO, 128), F32)
    k_s[0, :, 0:HALO, :] = zeros
    v_s[0, :, 0:HALO, :] = zeros

    c_wv[0].wait()
    permute_qkv(2, 0, [0, 1])
    c_wv[1].wait()
    permute_qkv(2, 0, [2, 3])
    c_x0.wait()
    x0 = load_x(rows(0))
    xn0 = _ln(x0).astype(BF16)
    proj_kv(xn0, 2, 0, 0, HT, True)
    proj_kv(xn0, 2, 0, HT, T, True)
    c_wk.wait()
    c_x1.wait()
    x1 = load_x(rows(1))
    xn1 = _ln(x1).astype(BF16)
    v_s[1, :, 0:HALO, :] = v_s[0, :, T:T + HALO, :]
    proj_kv(xn1, 2, 1, 0, HT, True)
    proj_kv(xn1, 2, 1, HT, T, True)
    permute_qkv(1, 1)
    proj_kv(xn0, 1, 0, 0, HT, True)
    c_wq.wait()
    c_wo.wait()
    c_b1.wait()
    c_b2.wait()
    proj_kv(xn0, 1, 0, HT, T, True)
    k_s[1, :, 0:HALO, :] = k_s[0, :, T:T + HALO, :]
    proj_kv(xn1, 1, 1, 0, HT, True)
    permute_qkv(0, 0)
    proj_q(xn0, 0, 0, HT, True)
    proj_q(xn0, 0, HT, T, True)
    proj_kv(xn1, 1, 1, HT, T, True)
    proj_q(xn1, 1, 0, HT, True)
    proj_q(xn1, 1, HT, T, True)
    permute_wo(1)
    b1f[...] = b1_s[...].astype(F32).reshape(1, F)
    b2f[...] = b2_s[...].astype(F32).reshape(1, D)
    attention(0, 0, STAGE_P)
    if "px" in OPT:
        x0 = load_x(pl.ds(0, T))
    x0a = attn_out(x0[0:HT], 0, 0, HT)
    y0a = ln2(x0a)
    x0b = attn_out(x0[HT:T], 0, HT, T)
    c_w1.wait()
    c_w2.wait()
    h0a = mlp1(y0a, first=True)
    h0b = mlp1(ln2(x0b), first=True)
    x0 = jnp.concatenate([x0a, x0b], axis=0)
    h0 = jnp.concatenate([h0a, h0b], axis=0)
    x0 = mlp2(x0, h0, first=True)
    w1_p[...] = _pack(w1_s[...])
    for p in (0, 2):
        for n0 in range(0, D, 128):
            wqkv_n[p // 2, :, n0:n0 + 128] = _pack(_unpack(wqkv_t[p, n0 // 2:(n0 + 128) // 2, :]).T)
    w2_p[...] = _pack(w2_s[...])
    attention(1, None, STAGE_P)
    if "px" in OPT:
        x1 = load_x(pl.ds(T, T))
    x1 = attn_out(x1, 1)
    xres[0] = x0
    xn_s[...] = _pack(_ln(x0).astype(BF16))
    xres[1] = x1
    c_xr.wait()

    def unit(xa, xna, slot, tile, xb, stage, last=False):
        proj_kv(xna, 2, slot)
        proj_kv(xna, 1, slot)
        proj_q(xna, slot, QCUTS[0], QCUTS[1])
        y = ln2(xb)
        ha = mlp1(y, W1CUTS[0], W1CUTS[1])
        proj_q(xna, slot, QCUTS[1], QCUTS[2])
        hb = mlp1(y, W1CUTS[1], W1CUTS[2])
        proj_q(xna, slot, QCUTS[2], QCUTS[3])
        h = jnp.concatenate([ha, hb], axis=1)
        if not last:
            z = mlp2(xb, h)
            attention(slot, tile, stage)
            return attn_out(xa, slot), z
        za = mlp2(xb, h, 0, D // 2)
        attention(slot, tile, stage)
        xa = attn_out(xa, slot)
        zb = mlp2(xb, h, D // 2, D)
        return xa, jnp.concatenate([za, zb], axis=1)

    def unit_x(t, stage):
        set_halo(0, 0)
        return unit(xres[0], _unpack(xn_s[...]), 0, None if isinstance(t, int) else t, xres[1], stage)

    def emit(o, rr):
        o_s[rr, :] = o.astype(BF16)
        out_copy(rr).start()

    def body(t, carry):
        xa, z = unit_x(t, STAGE_L)
        if "z" in OPT:
            xres[3] = z
            z = xres[3]
        xnc = _ln(load_x(rows(t + 2))).astype(BF16)
        xc = load_x(rows(t, T, 2 * T))
        set_halo(1, 1)
        xres[2] = xa
        xc, o = unit(xc, xnc, 1, None, xres[2], STAGE_L)
        emit(o, rows(t))
        xres[1] = xc
        xres[0] = z
        xn_s[...] = _pack(_ln(z).astype(BF16))
        return carry

    jax.lax.fori_loop(0, NITER, body, 0)

    xa, z = unit_x(NT - 2, STAGE_E)
    set_halo(1, 0)
    if "ex" in OPT:
        xres[2] = xa
        xa = xres[2]
        xres[3] = z
        z = xres[3]
    xc, o = unit(z, _ln(z).astype(BF16), 1, None, xa, STAGE_E, last=True)
    emit(o, rows(NT - 2))
    if "ex" in OPT:
        xres[1] = xc
        xc = xres[1]
    h = mlp1(ln2(xc))
    cuts = (0, 192, T)
    for i in range(len(cuts) - 1):
        emit(mlp2(xc[cuts[i]:cuts[i + 1]], h[cuts[i]:cuts[i + 1]]),
             rows(NT - 1, cuts[i + 1] - cuts[i], cuts[i]))
    for t in list(range(NITER)) + [NT - 2]:
        out_copy(rows(t)).wait()
    for i in range(len(cuts) - 1):
        out_copy(rows(NT - 1, cuts[i + 1] - cuts[i], cuts[i])).wait()


@jax.jit
def pallas_interleave_layers__sliding_local_dilated__mixer_channel_mlp__prompt_kernel(
    A_x, A_wqkv, A_wo, B_x, B_w1, B_b1, B_w2, B_b2,
):
    del B_x
    any_spec = pl.BlockSpec(memory_space=pl.ANY)
    out = pl.pallas_call(
        _kernel,
        in_specs=[any_spec] * 7,
        out_specs=any_spec,
        out_shape=jax.ShapeDtypeStruct((S, D), BF16),
        scratch_shapes=[
            pltpu.VMEM((S, D), BF16),
            pltpu.VMEM((3, D, D), BF16),
            pltpu.VMEM((D, D), BF16),
            pltpu.VMEM((2, 4, H * PITCH, 128), F32),
            pltpu.VMEM((3, D // 2, D), U32),
            pltpu.VMEM((2, D // 2, D), U32),
            pltpu.VMEM((D // 2, D), U32),
            pltpu.VMEM((F, D), BF16),
            pltpu.VMEM((F, D), BF16),
            pltpu.VMEM((F // 2, D), U32),
            pltpu.VMEM((F // 2, D), U32),
            pltpu.VMEM((F,), BF16),
            pltpu.VMEM((D,), BF16),
            pltpu.VMEM((1, F), F32),
            pltpu.VMEM((1, D), F32),
            pltpu.VMEM((2, 4, HALO + T, 128), F32),
            pltpu.VMEM((2, 4, HALO + T, 128), F32),
            pltpu.VMEM((2, T, D), F32),
            pltpu.VMEM((4, W, T, 128), F32),
            pltpu.VMEM((2, T // 2, D), U32),
            pltpu.VMEM((4, T, D), F32),
            pltpu.VMEM((T // 2, D), U32),
            pltpu.VMEM((S, D), BF16),
            pltpu.SemaphoreType.DMA((7,)),
            pltpu.SemaphoreType.DMA((1,)),
        ],
        compiler_params=pltpu.CompilerParams(vmem_limit_bytes=100 * 1024 * 1024),
    )(A_x.reshape(S, D), A_wqkv, A_wo, B_w1.T, B_b1, B_w2, B_b2)
    return out.reshape(1, S, D)
```

```python
import jax
import jax.numpy as jnp
import jax.experimental.pallas as pl
import jax.experimental.pallas.tpu as pltpu

S, D, F = 2048, 512, 1376
H, DH, W, DIL = 32, 16, 8, 2
HALO = 16
T = 256
HT = T // 2
NT = S // T
RC = 16
PITCH = 20
EPS = 1e-5
F32 = jnp.float32
BF16 = jnp.bfloat16
U32 = jnp.uint32
NT_DIMS = (((1,), (1,)), ((), ()))

QCUTS = (0, 64, 128, T)
W1CUT = 512
STAGE_PROLOGUE, STAGE_LOOP, STAGE_EPILOGUE = (1, 2, 3), (2, 3), ()


def _ln(x):
    m = jnp.mean(x, axis=-1, keepdims=True)
    xc = x - m
    v = jnp.mean(xc * xc, axis=-1, keepdims=True)
    return xc * jax.lax.rsqrt(v + EPS)


def _gelu(x):
    c = 0.7978845608028654
    return 0.5 * x * (1.0 + jnp.tanh(c * (x + 0.044715 * (x * x * x))))


def _pack(x):
    return pltpu.bitcast(x, U32)


def _unpack(x):
    return pltpu.bitcast(x, BF16)


def _dot(a, b):
    return jnp.dot(a, b, preferred_element_type=F32)


def _dot_nt(a, b):
    return jax.lax.dot_general(a, b, NT_DIMS, preferred_element_type=F32)


def _kernel(x_hbm, wqkv_hbm, wo_hbm, w1t_hbm, b1_hbm, w2_hbm, b2_hbm, out_hbm,
            xin, wraw, woraw, wt32, wqkv_t, wqkv_n, wo_p, w1_s, w2_s, w1_p, w2_p,
            b1_s, b2_s, b1f, b2f, k_s, v_s, q_s, l_s, a_s, xres, xn_s, o_s,
            sem_in, sem_out):
    def cp(src, dst, i):
        return pltpu.make_async_copy(src, dst, sem_in.at[i])

    c_wv = [cp(wqkv_hbm.at[pl.ds(c * 256, 256), pl.ds(2 * D, D)],
               wraw.at[2, pl.ds(c * 256, 256), :], c) for c in range(2)]
    c_x0 = cp(x_hbm.at[pl.ds(0, T), :], xin.at[pl.ds(0, T), :], 2)
    c_wk = cp(wqkv_hbm.at[:, pl.ds(D, D)], wraw.at[1], 3)
    c_x1 = cp(x_hbm.at[pl.ds(T, T), :], xin.at[pl.ds(T, T), :], 3)
    c_wq = cp(wqkv_hbm.at[:, pl.ds(0, D)], wraw.at[0], 4)
    c_wo = cp(wo_hbm, woraw, 4)
    c_b1 = cp(b1_hbm, b1_s, 4)
    c_b2 = cp(b2_hbm, b2_s, 4)
    c_w1 = cp(w1t_hbm, w1_s, 5)
    c_w2 = cp(w2_hbm, w2_s, 5)
    c_xr = cp(x_hbm.at[pl.ds(2 * T, S - 2 * T), :], xin.at[pl.ds(2 * T, S - 2 * T), :], 6)
    for c in c_wv + [c_x0, c_wk, c_x1, c_wq, c_wo, c_b1, c_b2, c_w1, c_w2, c_xr]:
        c.start()

    def rows(tile, n=T, off=0):
        r0 = tile * T
        if not isinstance(tile, int):
            r0 = pl.multiple_of(r0, T)
        return pl.ds(r0 + off, n)

    def out_copy(rr):
        return pltpu.make_async_copy(o_s.at[rr, :], out_hbm.at[rr, :], sem_out.at[0])

    def scatter_heads(buf, c, wt):
        for h in range(H):
            wt32[buf, c, h * PITCH:h * PITCH + DH, :] = wt[h * DH:(h + 1) * DH, :]

    def gather_heads(buf, c, d):
        return wt32[buf, c, pl.ds(d, H, stride=PITCH), :]

    def permute_qkv(p, buf, chunks=range(4)):
        for c in chunks:
            scatter_heads(buf, c, wraw[p, c * 128:(c + 1) * 128, :].astype(F32).T)
        for d in range(DH):
            for c in chunks:
                blk = gather_heads(buf, c, d)
                if p == 0:
                    blk = blk * (DH ** -0.5)
                wqkv_t[p, d * H // 2:(d + 1) * H // 2, c * 128:(c + 1) * 128] = _pack(blk.astype(BF16))

    def permute_wo(buf):
        for c in range(4):
            scatter_heads(buf, c, woraw[:, c * 128:(c + 1) * 128].astype(F32))
        for d in range(DH):
            for c in range(4):
                wo_p[d * H // 2:(d + 1) * H // 2, c * 128:(c + 1) * 128] = _pack(
                    gather_heads(buf, c, d).astype(BF16))

    def make_nn(p):
        for n0 in range(0, D, 128):
            wqkv_n[p // 2, :, n0:n0 + 128] = _pack(_unpack(wqkv_t[p, n0 // 2:(n0 + 128) // 2, :]).T)

    def proj(xn, p, first):
        if first or p == 1:
            return _dot_nt(xn, _unpack(wqkv_t[p]))
        return _dot(xn, _unpack(wqkv_n[p // 2]))

    def proj_kv(xn, p, slot, r0=0, r1=T, first=False):
        dst = k_s if p == 1 else v_s
        y = proj(xn[r0:r1], p, first)
        for t in range(4):
            dst[slot, t, HALO + r0:HALO + r1, :] = y[:, 128 * t:128 * (t + 1)]

    def proj_q(xn, slot, r0, r1, first=False):
        q_s[slot, r0:r1, :] = proj(xn[r0:r1], 0, first)

    def attention(slot, tile, stage):
        def through(i, w, r, val):
            if i not in stage:
                return val
            l_s[i - 1, w, r:r + RC, :] = val
            return l_s[i - 1, w, r:r + RC, :]

        for r in range(0, T, RC):
            q = [q_s[slot, r:r + RC, 128 * t:128 * (t + 1)] for t in range(4)]
            logits = []
            for w in range(W):
                st = HALO + r - DIL * w
                p = q[0] * k_s[slot, 0, st:st + RC, :]
                for t in range(1, 4):
                    p = p + q[t] * k_s[slot, t, st:st + RC, :]
                p = p + pltpu.roll(p, 64, 1)
                p = through(1, w, r, p)
                p = p + pltpu.roll(p, 32, 1)
                if tile is not None and r < HALO and w > 0:
                    row = tile * T + r + jax.lax.broadcasted_iota(jnp.int32, (RC, 128), 0)
                    p = jnp.where(row >= DIL * w, p, -1e9)
                logits.append(through(2, w, r, p))
            m = logits[0]
            for w in range(1, W):
                m = jnp.maximum(m, logits[w])
            e = [through(3, w, r, jnp.exp(logits[w] - m)) for w in range(W)]
            den = e[0]
            for w in range(1, W):
                den = den + e[w]
            inv = 1.0 / den
            for t in range(4):
                acc = None
                for w in range(W):
                    st = HALO + r - DIL * w
                    term = e[w] * v_s[slot, t, st:st + RC, :]
                    acc = term if acc is None else acc + term
                a_s[slot, r // 2:(r + RC) // 2, 128 * t:128 * (t + 1)] = _pack((acc * inv).astype(BF16))

    def attn_out(x, slot, r0=0, r1=T):
        return x + _dot(_unpack(a_s[slot, r0 // 2:r1 // 2, :]), _unpack(wo_p[...]))

    def ln2(x):
        return _ln(_ln(x)).astype(BF16)

    def mlp1(y, a=0, b=F, first=False):
        w = w1_s[a:b, :] if first else _unpack(w1_p[a // 2:b // 2, :])
        return _gelu(_dot_nt(y, w) + b1f[:, a:b]).astype(BF16)

    def mlp2(x, h, a=0, b=D):
        return x[:, a:b] + _dot(h, _unpack(w2_p[:, a:b])) + b2f[:, a:b]

    def load_x(rr):
        return xin[rr, :].astype(F32)

    def set_halo(slot, src_slot):
        k_s[slot, :, 0:HALO, :] = k_s[src_slot, :, T:T + HALO, :]
        v_s[slot, :, 0:HALO, :] = v_s[src_slot, :, T:T + HALO, :]

    zeros = jnp.zeros((4, HALO, 128), F32)
    k_s[0, :, 0:HALO, :] = zeros
    v_s[0, :, 0:HALO, :] = zeros

    c_wv[0].wait()
    permute_qkv(2, 0, [0, 1])
    c_wv[1].wait()
    permute_qkv(2, 0, [2, 3])
    c_x0.wait()
    x0 = load_x(rows(0))
    xn0 = _ln(x0).astype(BF16)
    proj_kv(xn0, 2, 0, 0, HT, True)
    proj_kv(xn0, 2, 0, HT, T, True)
    c_wk.wait()
    c_x1.wait()
    x1 = load_x(rows(1))
    xn1 = _ln(x1).astype(BF16)
    v_s[1, :, 0:HALO, :] = v_s[0, :, T:T + HALO, :]
    proj_kv(xn1, 2, 1, 0, HT, True)
    proj_kv(xn1, 2, 1, HT, T, True)
    permute_qkv(1, 1)
    proj_kv(xn0, 1, 0, 0, HT, True)
    c_wq.wait()
    c_wo.wait()
    c_b1.wait()
    c_b2.wait()
    proj_kv(xn0, 1, 0, HT, T, True)
    k_s[1, :, 0:HALO, :] = k_s[0, :, T:T + HALO, :]
    proj_kv(xn1, 1, 1, 0, HT, True)
    permute_qkv(0, 0)
    proj_q(xn0, 0, 0, HT, True)
    proj_q(xn0, 0, HT, T, True)
    proj_kv(xn1, 1, 1, HT, T, True)
    make_nn(0)
    proj_q(xn1, 1, 0, HT, True)
    proj_q(xn1, 1, HT, T)
    permute_wo(1)
    b1f[...] = b1_s[...].astype(F32).reshape(1, F)
    b2f[...] = b2_s[...].astype(F32).reshape(1, D)
    attention(0, 0, STAGE_PROLOGUE)
    x0a = attn_out(x0[0:HT], 0, 0, HT)
    y0a = ln2(x0a)
    x0b = attn_out(x0[HT:T], 0, HT, T)
    c_w1.wait()
    c_w2.wait()
    h0a = mlp1(y0a, first=True)
    w1_p[...] = _pack(w1_s[...])
    h0b = mlp1(ln2(x0b))
    x0 = jnp.concatenate([x0a, x0b], axis=0)
    h0 = jnp.concatenate([h0a, h0b], axis=0)
    w2_p[...] = _pack(w2_s[...])
    x0 = mlp2(x0, h0)
    make_nn(2)
    attention(1, None, STAGE_PROLOGUE)
    x1 = attn_out(x1, 1)
    xres[0] = x0
    xn_s[...] = _pack(_ln(x0).astype(BF16))
    xres[1] = x1
    c_xr.wait()

    def unit(xa, xna, slot, tile, xb, stage, last=False):
        proj_kv(xna, 2, slot)
        proj_kv(xna, 1, slot)
        proj_q(xna, slot, QCUTS[0], QCUTS[1])
        y = ln2(xb)
        ha = mlp1(y, 0, W1CUT)
        proj_q(xna, slot, QCUTS[1], QCUTS[2])
        hb = mlp1(y, W1CUT, F)
        proj_q(xna, slot, QCUTS[2], QCUTS[3])
        h = jnp.concatenate([ha, hb], axis=1)
        if not last:
            z = mlp2(xb, h)
            attention(slot, tile, stage)
            return attn_out(xa, slot), z
        za = mlp2(xb, h, 0, D // 2)
        attention(slot, tile, stage)
        xa = attn_out(xa, slot)
        zb = mlp2(xb, h, D // 2, D)
        return xa, jnp.concatenate([za, zb], axis=1)

    def unit_x(t, stage):
        set_halo(0, 0)
        return unit(xres[0], _unpack(xn_s[...]), 0, None if isinstance(t, int) else t, xres[1], stage)

    def emit(o, rr):
        o_s[rr, :] = o.astype(BF16)
        out_copy(rr).start()

    def body(t, carry):
        xa, z = unit_x(t, STAGE_LOOP)
        xnc = _ln(load_x(rows(t + 2))).astype(BF16)
        xc = load_x(rows(t, T, 2 * T))
        set_halo(1, 1)
        xres[2] = xa
        xc, o = unit(xc, xnc, 1, None, xres[2], STAGE_LOOP)
        emit(o, rows(t))
        xres[1] = xc
        xres[0] = z
        xn_s[...] = _pack(_ln(z).astype(BF16))
        return carry

    jax.lax.fori_loop(0, NT - 2, body, 0)

    xa, z = unit_x(NT - 2, STAGE_EPILOGUE)
    set_halo(1, 0)
    xres[2] = xa
    xres[3] = z
    z = xres[3]
    xc, o = unit(z, _ln(z).astype(BF16), 1, None, xres[2], STAGE_EPILOGUE, last=True)
    emit(o, rows(NT - 2))
    xres[1] = xc
    xc = xres[1]
    h = mlp1(ln2(xc))
    cuts = (0, 192, T)
    for i in range(len(cuts) - 1):
        emit(mlp2(xc[cuts[i]:cuts[i + 1]], h[cuts[i]:cuts[i + 1]]),
             rows(NT - 1, cuts[i + 1] - cuts[i], cuts[i]))
    for t in range(NT - 1):
        out_copy(rows(t)).wait()
    for i in range(len(cuts) - 1):
        out_copy(rows(NT - 1, cuts[i + 1] - cuts[i], cuts[i])).wait()


@jax.jit
def pallas_interleave_layers__sliding_local_dilated__mixer_channel_mlp__prompt_kernel(
    A_x: jax.Array,
    A_wqkv: jax.Array,
    A_wo: jax.Array,
    B_x: jax.Array,
    B_w1: jax.Array,
    B_b1: jax.Array,
    B_w2: jax.Array,
    B_b2: jax.Array,
):
    del B_x
    any_spec = pl.BlockSpec(memory_space=pl.ANY)
    out = pl.pallas_call(
        _kernel,
        in_specs=[any_spec] * 7,
        out_specs=any_spec,
        out_shape=jax.ShapeDtypeStruct((S, D), BF16),
        scratch_shapes=[
            pltpu.VMEM((S, D), BF16),
            pltpu.VMEM((3, D, D), BF16),
            pltpu.VMEM((D, D), BF16),
            pltpu.VMEM((2, 4, H * PITCH + DH, 128), F32),
            pltpu.VMEM((3, D // 2, D), U32),
            pltpu.VMEM((2, D // 2, D), U32),
            pltpu.VMEM((D // 2, D), U32),
            pltpu.VMEM((F, D), BF16),
            pltpu.VMEM((F, D), BF16),
            pltpu.VMEM((F // 2, D), U32),
            pltpu.VMEM((F // 2, D), U32),
            pltpu.VMEM((F,), BF16),
            pltpu.VMEM((D,), BF16),
            pltpu.VMEM((1, F), F32),
            pltpu.VMEM((1, D), F32),
            pltpu.VMEM((2, 4, HALO + T, 128), F32),
            pltpu.VMEM((2, 4, HALO + T, 128), F32),
            pltpu.VMEM((2, T, D), F32),
            pltpu.VMEM((3, W, T, 128), F32),
            pltpu.VMEM((2, T // 2, D), U32),
            pltpu.VMEM((4, T, D), F32),
            pltpu.VMEM((T // 2, D), U32),
            pltpu.VMEM((S, D), BF16),
            pltpu.SemaphoreType.DMA((7,)),
            pltpu.SemaphoreType.DMA((1,)),
        ],
        compiler_params=pltpu.CompilerParams(vmem_limit_bytes=100 * 1024 * 1024),
    )(A_x.reshape(S, D), A_wqkv, A_wo, B_w1.T, B_b1, B_w2, B_b2)
    return out.reshape(1, S, D)
```
